```python
import os as _os
_os.environ.setdefault("JAX_PLATFORMS", "cpu")
import jax
import jax.numpy as jnp

def _softmax(x, axis=-1):
    return jax.nn.softmax(x, axis=axis)
def _gelu(x):
    return jax.nn.gelu(x, approximate=True)
def _silu(x):
    return jax.nn.silu(x)
def _sigmoid(x):
    return jax.nn.sigmoid(x)
def _layernorm(x, axis=-1, eps=1e-5):
    m = jnp.mean(x, axis=axis, keepdims=True)
    v = jnp.var(x, axis=axis, keepdims=True)
    return (x - m) / jnp.sqrt(v + eps)
def _scatter_add(tgt, idx, src, axis=0):
    return tgt.at[idx].add(src)
def _segment_sum(src, seg, n):
    return jax.ops.segment_sum(src, seg, n)
class _Rng:
    def __init__(self, key):
        self._k = key
    def _next(self):
        self._k, sub = jax.random.split(self._k)
        return sub
    def normal(self, shape):
        return jax.random.normal(self._next(), shape, dtype=jnp.bfloat16)
    def randint(self, lo, hi, shape):
        return jax.random.randint(self._next(), shape, lo, hi, dtype=jnp.int32)
    def uniform(self, shape, lo=0.0, hi=1.0):
        return jax.random.uniform(self._next(), shape, jnp.bfloat16, lo, hi)
    def permutation(self, n):
        return jax.random.permutation(self._next(), n)


kernel_name = 'sequential_preLN__mha_block__moe_arch_mod__prompt'

def setup_inputs():
    _rng = _Rng(jax.random.key(int.from_bytes(__import__("os").urandom(4), "little")))
    _w = (lambda a: (lambda t: t.astype(jnp.bfloat16) if jnp.issubdtype(t.dtype, jnp.floating) else t)(jnp.asarray(a)))
    def _A_setup():
        B, S, D, H = 1, 2048, 640, 32
        return {
            "x": _w((lambda *s: _rng.normal(s) * 0.05)(B, S, D)),
            "wqkv": _w((lambda *s: _rng.normal(s) * 0.05)(D, 3 * D)),
            "wo": _w((lambda *s: _rng.normal(s) * 0.05)(D, D)),
        }
    _A_in = _A_setup()

    def _B_setup():
        B, S, D, F, C = 1, 2048, 640, 1536, 1
        return {
            "x": _w((lambda *s: _rng.normal(s) * 0.05)(B, S, D)),
            "w_r": _w((lambda *s: _rng.normal(s) * 0.05)(D)),
            "w_gate": _w((lambda *s: _rng.normal(s) * 0.05)(D, F)),
            "w_up": _w((lambda *s: _rng.normal(s) * 0.05)(D, F)),
            "w_down": _w((lambda *s: _rng.normal(s) * 0.05)(F, D)),
        }
    _B_in = _B_setup()

    return {
        "A_x": _A_in["x"],
        "A_wqkv": _A_in["wqkv"],
        "A_wo": _A_in["wo"],
        "B_x": _B_in["x"],
        "B_w_r": _B_in["w_r"],
        "B_w_gate": _B_in["w_gate"],
        "B_w_up": _B_in["w_up"],
        "B_w_down": _B_in["w_down"],
    }

def reference(A_x, A_wqkv, A_wo, B_x, B_w_r, B_w_gate, B_w_up, B_w_down):
    def _A_ref(x, wqkv, wo):
        B, S, D = x.shape
        H = 32
        Dh = D // H
        qkv = (lambda x, *d: x.transpose(*d))((x @ wqkv).reshape(B, S, 3, H, Dh), 2, 0, 3, 1, 4)
        q, k, v = qkv[0], qkv[1], qkv[2]
        scores = jnp.einsum("bhqd,bhkd->bhqk", q, k) * (Dh ** -0.5)
        p = _softmax(scores, axis=-1)
        o = jnp.einsum("bhqk,bhkd->bhqd", p, v)
        return (lambda x, *d: x.transpose(*d))(o, 0, 2, 1, 3).reshape(B, S, D) @ wo

    def _B_ref(x, w_r, w_gate, w_up, w_down):
        B, S, D = x.shape
        C = 1
        r = x @ w_r
        idx = jnp.argsort(-r, axis=-1)[:, :C]
        idx_e = jnp.repeat(idx.reshape(B, C, 1), D, axis=2)
        x_sel = jnp.take_along_axis(x, idx_e, axis=1)
        g = _silu(x_sel @ w_gate)
        u = x_sel @ w_up
        y = (g * u) @ w_down
        r_sel = _sigmoid(jnp.take_along_axis(r, idx, axis=1))
        y = y * r_sel.reshape(B, C, 1)
        b_off = (jnp.arange(B) * S).reshape(B, 1)
        flat_idx = (idx + b_off).reshape(B * C)
        zero = (x * 0.0).reshape(B * S, D)
        upd = _scatter_add(zero, flat_idx, y.reshape(B * C, D), axis=0)
        return x + upd.reshape(B, S, D)

    x = A_x
    h = x + _A_ref(_layernorm(x, axis=-1), A_wqkv, A_wo)
    h2 = h + _B_ref(_layernorm(h, axis=-1), B_w_r, B_w_gate, B_w_up, B_w_down)
    return h2
```

```python
import functools
import os

import jax
import jax.numpy as jnp
import numpy as np
from jax.experimental import pallas as pl
from jax.experimental.pallas import tpu as pltpu

F32 = jnp.float32
BF16 = jnp.bfloat16
I32 = jnp.int32

H = 32
LANES = 128
QB = 512
NQ = QB // LANES
VR = 24

G = int(os.environ.get("KG", "1"))
R1 = int(os.environ.get("KR1", "256"))
R3 = int(os.environ.get("KR3", "256"))

NT = (((1,), (1,)), ((), ()))


def _rb(x):
    return x.astype(BF16).astype(F32)


def _layernorm(xf, d):
    mean = jnp.sum(xf, axis=-1, keepdims=True) / d
    c = xf - mean
    var = jnp.sum(c * c, axis=-1, keepdims=True) / d
    eps = np.float32(np.asarray(1e-5, dtype=jnp.bfloat16))
    den = _rb(jnp.sqrt(_rb(_rb(var) + eps)))
    return (_rb(xf - _rb(mean)) * (1.0 / den)).astype(BF16)


def _head_geometry(h, dh):
    col = h * dh
    tile, lo = col // LANES, col % LANES
    straddle = lo + dh > LANES
    return tile, lo, straddle


def kernel(z_ref, x_ref, wqkv_ref, wo_ref, wr_ref, wg_ref, wu_ref, wd_ref,
           out_ref,
           xn_s, wvt_s, qm_s, ks_s, vtw_s, s0, s1, m0, m1, ot_s, h_s, hn_s, bv_s, bi_s,
           *, S, D, DH, FF):
    NTILE = D // LANES
    straddlers = [h for h in range(H) if _head_geometry(h, DH)[2]]
    scale = float(np.float32(np.asarray(DH ** -0.5, dtype=jnp.bfloat16)))
    C = np.float32(scale * np.log2(np.e))

    wvt_s[...] = wqkv_ref[:, 2 * D:3 * D].T

    def proj_step(i, carry):
        r0 = pl.multiple_of(i * R1, R1)
        rows = pl.ds(r0, R1)
        xn = _layernorm(x_ref[rows, :].astype(F32), D)
        lane = jax.lax.broadcasted_iota(I32, (R1, LANES), 1)
        qk = jnp.dot(xn, wqkv_ref[:, 0:2 * D], preferred_element_type=F32)
        qt = [qk[:, t * LANES:(t + 1) * LANES].astype(BF16) for t in range(NTILE)]
        kt = [qk[:, D + t * LANES:D + (t + 1) * LANES].astype(BF16) for t in range(NTILE)]
        zero = jnp.zeros((R1, LANES), BF16)
        for t in range(NTILE):
            ks_s[t, rows, :] = kt[t]
        for h in range(H):
            t, lo, st = _head_geometry(h, DH)
            if st:
                qsl = jnp.where(lane >= lo, qt[t], qt[t + 1])
                ks_s[NTILE + straddlers.index(h), rows, :] = jnp.where(lane >= lo, kt[t], kt[t + 1])
            else:
                qsl = qt[t]
            mask = ((lane - lo) & (LANES - 1)) < DH
            qm_s[h, rows, :] = jnp.where(mask, qsl, zero)
        vt = _rb(jax.lax.dot_general(wvt_s[...], xn, NT, preferred_element_type=F32))
        sub = jax.lax.broadcasted_iota(I32, (VR, LANES), 0)
        for h in range(H):
            w0 = (h * DH) // 8 * 8
            off = h * DH - w0
            inhead = (sub >= off) & (sub < off + DH)
            for c in range(R1 // LANES):
                win = vt[w0:w0 + VR, c * LANES:(c + 1) * LANES]
                vtw_s[h, i * (R1 // LANES) + c] = jnp.where(inhead, win, 1.0)
        return carry

    jax.lax.fori_loop(0, S // R1, proj_step, 0)

    NKT = S // LANES
    NQB = S // QB
    off = pl.multiple_of(jnp.clip(z_ref[0], 0, 1) * 8, 8)

    def head_slab(h):
        col = h * DH
        t = col >> 7
        lo = col & (LANES - 1)
        return jnp.where(lo + DH > LANES, NTILE + t, t)

    def qk_start(h, qb):
        return dict(slab=head_slab(h), h=h, q0=pl.multiple_of(qb * QB, QB), ms=[None] * NQ)

    def qk_chunk(st, s_ref, kc):
        q = qm_s[st["h"], pl.ds(st["q0"], QB), :]
        k = ks_s[st["slab"], kc * LANES:(kc + 1) * LANES, :]
        s = jax.lax.dot_general(k, q, NT, preferred_element_type=F32)
        for j in range(NQ):
            sj = s[:, j * LANES:(j + 1) * LANES]
            s_ref[j, kc * LANES:(kc + 1) * LANES, :] = sj
            pm = jnp.max(sj.reshape(LANES // 8, 8, LANES), axis=0)
            st["ms"][j] = pm if st["ms"][j] is None else jnp.maximum(st["ms"][j], pm)

    def qk_finish(st, m_ref):
        for j in range(NQ):
            m_ref[j] = jnp.broadcast_to(jnp.max(st["ms"][j], axis=0, keepdims=True), (8, LANES))

    def ep_start(h, m_ref):
        return dict(h=h, m=[m_ref[j] for j in range(NQ)], acc=[None] * NQ)

    def ep_chunk(st, s_ref, kc):
        vt = vtw_s[st["h"], kc]
        for j in range(NQ):
            s = s_ref[j, pl.ds(off + kc * LANES, LANES), :]
            p = jnp.exp2((s.reshape(LANES // 8, 8, LANES) - st["m"][j][None]) * C)
            p = p.reshape(LANES, LANES).astype(BF16)
            d = jnp.dot(vt, p, preferred_element_type=F32)
            st["acc"][j] = d if st["acc"][j] is None else st["acc"][j] + d

    def ep_finish(st, pair, parity, qb):
        for j in range(NQ):
            acc = st["acc"][j]
            q0 = pl.multiple_of(qb * QB + j * LANES, LANES)
            if parity == 0:
                l = acc[DH:DH + 1, :]
                ot_s[pair, 0:DH, pl.ds(q0, LANES)] = acc[0:DH, :] * (1.0 / l)
            else:
                l = acc[0:1, :]
                ot_s[pair, DH:2 * DH, pl.ds(q0, LANES)] = acc[VR - DH:VR, :] * (1.0 / l)

    def both(nxt, cur, s_nxt, m_nxt, s_cur, m_cur):
        (hn, qbn), (pc, ec, qbc) = nxt, cur
        a = qk_start(hn, qbn)
        b = ep_start(2 * pc + ec, m_cur)
        for kc in range(NKT):
            qk_chunk(a, s_nxt, kc)
            ep_chunk(b, s_cur, kc)
        qk_finish(a, m_nxt)
        ep_finish(b, pc, ec, qbc)

    a = qk_start(0, 0)
    for kc in range(NKT):
        qk_chunk(a, s0, kc)
    qk_finish(a, m0)

    NGRP = NQB // G
    NIT = (H // 2) * NGRP

    def att_step(i, carry):
        pair = i // NGRP
        grp = i % NGRP
        i1 = jnp.minimum(i + 1, NIT - 1)
        pair1 = i1 // NGRP
        grp1 = i1 % NGRP
        for g in range(G):
            qb = grp * G + g
            both((2 * pair + 1, qb), (pair, 0, qb), s1, m1, s0, m0)
            if g + 1 < G:
                nxt = (2 * pair, qb + 1)
            else:
                nxt = (2 * pair1, grp1 * G)
            both(nxt, (pair, 1, qb), s0, m0, s1, m1)
        return carry

    jax.lax.fori_loop(0, NIT, att_step, 0)

    bv_s[...] = jnp.full((8, LANES), -jnp.inf, F32)
    bi_s[...] = jnp.zeros((8, LANES), I32)
    wr = wr_ref[...].astype(F32)

    def epi_step(i, carry):
        r0 = pl.multiple_of(i * R3, R3)
        rows = pl.ds(r0, R3)
        oT = ot_s[:, :, rows].reshape(D, R3).astype(BF16)
        attn = jnp.dot(oT.T, wo_ref[...], preferred_element_type=F32)
        h = _rb(x_ref[rows, :].astype(F32) + _rb(attn))
        hn = _layernorm(h, D).astype(F32)
        r = _rb(jnp.sum(hn * wr, axis=-1, keepdims=True))
        h_s[rows, :] = h
        hn_s[rows, :] = hn
        out_ref[rows, :] = (h + hn).astype(BF16)
        bv = bv_s[...]
        bi = bi_s[...]
        sub = jax.lax.broadcasted_iota(I32, (8, LANES), 0)
        for t in range(R3 // 8):
            rv = jnp.broadcast_to(r[t * 8:(t + 1) * 8, :], (8, LANES))
            ri = sub + (r0 + t * 8)
            upd = rv > bv
            bv = jnp.where(upd, rv, bv)
            bi = jnp.where(upd, ri, bi)
        bv_s[...] = bv
        bi_s[...] = bi
        return carry

    jax.lax.fori_loop(0, S // R3, epi_step, 0)

    bv = bv_s[...]
    bi = bi_s[...]
    vmax = jnp.max(bv)
    idx = jnp.min(jnp.where(bv == vmax, bi, S))
    idx = jnp.clip(idx, 0, S - 1)
    xsel = hn_s[pl.ds(idx, 1), :]
    hsel = h_s[pl.ds(idx, 1), :]
    xb = jnp.broadcast_to(xsel, (16, D)).astype(BF16)
    g = _rb(jnp.dot(xb, wg_ref[...], preferred_element_type=F32))
    u = _rb(jnp.dot(xb, wu_ref[...], preferred_element_type=F32))
    act = _rb(g * jax.nn.sigmoid(g))
    t = (act * u).astype(BF16)
    y = _rb(jnp.dot(t, wd_ref[...], preferred_element_type=F32))
    rsel = _rb(jax.nn.sigmoid(jnp.full((16, LANES), vmax, F32)))
    y = _rb(y * rsel[:, 0:1])
    newrow = (hsel + _rb(xsel + y)).astype(BF16)
    base = pl.multiple_of((idx // 16) * 16, 16)
    rowid = jax.lax.broadcasted_iota(I32, (16, D), 0) + base
    old = out_ref[pl.ds(base, 16), :]
    out_ref[pl.ds(base, 16), :] = jnp.where(rowid == idx, newrow, old)


def build(S, D, FF):
    DH = D // H
    n_str = len([h for h in range(H) if _head_geometry(h, DH)[2]])
    scratch = [
        pltpu.VMEM((S, D), BF16),
        pltpu.VMEM((D, D), BF16),
        pltpu.VMEM((H, S, LANES), BF16),
        pltpu.VMEM((D // LANES + n_str, S, LANES), BF16),
        pltpu.VMEM((H, S // LANES, VR, LANES), F32),
        pltpu.VMEM((NQ, S + 8, LANES), F32),
        pltpu.VMEM((NQ, S + 8, LANES), F32),
        pltpu.VMEM((NQ, 8, LANES), F32),
        pltpu.VMEM((NQ, 8, LANES), F32),
        pltpu.VMEM((H // 2, 2 * DH, S), F32),
        pltpu.VMEM((S, D), F32),
        pltpu.VMEM((S, D), F32),
        pltpu.VMEM((8, LANES), F32),
        pltpu.VMEM((8, LANES), I32),
    ]
    vm = pl.BlockSpec(memory_space=pltpu.VMEM)
    return pl.pallas_call(
        functools.partial(kernel, S=S, D=D, DH=DH, FF=FF),
        out_shape=jax.ShapeDtypeStruct((S, D), BF16),
        in_specs=[pl.BlockSpec(memory_space=pltpu.SMEM)] + [vm] * 7,
        out_specs=vm,
        scratch_shapes=scratch,
        compiler_params=pltpu.CompilerParams(vmem_limit_bytes=120 * 1024 * 1024),
        name="fused_block",
    )


@jax.jit
def pallas_sequential_preLN__mha_block__moe_arch_mod__prompt_kernel(
        A_x, A_wqkv, A_wo, B_x, B_w_r, B_w_gate, B_w_up, B_w_down):
    del B_x
    B, S, D = A_x.shape
    FF = B_w_gate.shape[1]
    out = build(S, D, FF)(
        jnp.zeros((1,), I32),
        A_x.reshape(S, D), A_wqkv, A_wo, B_w_r.reshape(1, D), B_w_gate, B_w_up, B_w_down)
    return out.reshape(B, S, D)
```

```python
import functools
import os

import jax
import jax.numpy as jnp
import numpy as np
from jax.experimental import pallas as pl
from jax.experimental.pallas import tpu as pltpu

F32 = jnp.float32
BF16 = jnp.bfloat16
I32 = jnp.int32

H = 32
LANES = 128
QB = 512
NQ = QB // LANES
VR = 24

G = int(os.environ.get("KG", "4"))
LAG = int(os.environ.get("KLAG", "1"))
R1 = int(os.environ.get("KR1", "256"))
R3 = int(os.environ.get("KR3", "128"))
U1 = int(os.environ.get("KU1", "1"))
U3 = int(os.environ.get("KU3", "16"))
NFIRST = int(os.environ.get('KNF', '2'))
LATE = int(os.environ.get('KLATE', '1'))
DEPT = int(os.environ.get('KDEP', '-1'))
WR1D = int(os.environ.get('KWR1D', '1'))
FOLD = int(os.environ.get("KFOLD", "1"))

NT = (((1,), (1,)), ((), ()))


def _rb(x):
    return x.astype(BF16).astype(F32)


def _compact(col):
    r = col.shape[0]
    v = jnp.broadcast_to(col, (r, LANES)).reshape(r // 8, 8, LANES)
    lane = jax.lax.broadcasted_iota(I32, (8, LANES), 1)
    out = []
    for n in range(r // LANES):
        parts = [v[16 * n + g] for g in range(16)]
        width = 8
        while len(parts) > 1:
            m = (lane & width) != 0
            parts = [jnp.where(m, parts[i + 1], parts[i]) for i in range(0, len(parts), 2)]
            width *= 2
        out.append(parts[0])
    return out


def _expand(vregs):
    rows = [jnp.broadcast_to(c[:, 8 * g:8 * g + 1], (8, LANES)) for c in vregs for g in range(16)]
    return jnp.concatenate(rows, axis=0)


def _layernorm(xf, d):
    inv_d = np.float32(1.0 / d)
    mean = jnp.sum(xf, axis=-1, keepdims=True) * inv_d
    c = xf - mean
    ssq = jnp.sum(c * c, axis=-1, keepdims=True)
    eps = np.float32(np.asarray(1e-5, dtype=jnp.bfloat16))
    rcp = _expand([1.0 / _rb(jnp.sqrt(_rb(_rb(v * inv_d) + eps))) for v in _compact(ssq)])
    dev = _rb(xf - _rb(mean))
    rcp = jnp.concatenate([rcp] * (d // LANES), axis=1)
    return (dev * rcp).astype(BF16)


def _head_geometry(h, dh):
    col = h * dh
    tile, lo = col // LANES, col % LANES
    straddle = lo + dh > LANES
    return tile, lo, straddle


SCOPES = int(os.environ.get('KSCOPES', '0'))
import contextlib
def scope(name):
    return jax.named_scope(name) if SCOPES else contextlib.nullcontext()


def kernel(z_hbm, x_hbm, wqkv_hbm, wo_hbm, wr_hbm, wg_hbm, wu_hbm, wd_hbm,
           out_hbm,
           z_s, x_s, wqkv_s, wo_s, wr_s, wg_s, wu_s, wd_s, out_s, patch_s,
           wvt_s, qm_s, ks_s, vtw_s, s0a, s0b, s1a, s1b, m0, m1, ot_s, h_s, hn_s, bv_s, bi_s,
           sem_x, sem_w, sem_o,
           *, S, D, DH, FF):
    NTILE = D // LANES
    straddlers = [h for h in range(H) if _head_geometry(h, DH)[2]]
    scale = float(np.float32(np.asarray(DH ** -0.5, dtype=jnp.bfloat16)))
    C = np.float32(scale * np.log2(np.e))
    N1 = S // R1
    N3 = S // R3

    def x_copy(i):
        rows = pl.ds(pl.multiple_of(i * R1, R1), R1)
        return pltpu.make_async_copy(x_hbm.at[rows], x_s.at[rows], sem_x.at[i])

    def wqkv_copy(p):
        cols = pl.ds(p * D, D)
        return pltpu.make_async_copy(wqkv_hbm.at[:, cols], wqkv_s.at[:, cols], sem_w.at[p])

    w_late = [
        pltpu.make_async_copy(z_hbm, z_s, sem_w.at[3]),
        pltpu.make_async_copy(wo_hbm, wo_s, sem_w.at[4]),
        pltpu.make_async_copy(wr_hbm, wr_s, sem_w.at[5]),
        pltpu.make_async_copy(wg_hbm, wg_s, sem_w.at[6]),
        pltpu.make_async_copy(wu_hbm, wu_s, sem_w.at[7]),
        pltpu.make_async_copy(wd_hbm, wd_s, sem_w.at[8]),
    ]
    STAG = int(os.environ.get("KSTAG", "1"))
    x_copy(0).start()
    x_copy(1).start()
    wqkv_copy(0).start()

    def dma_stage2():
        wqkv_copy(1).start()
        wqkv_copy(2).start()

    def dma_stage3():
        for i in range(2, N1):
            x_copy(i).start()

    def dma_stage4():
        for c in w_late[:1] if LATE else w_late:
            c.start()

    if STAG == 0:
        dma_stage2()
        dma_stage3()
        dma_stage4()
    if STAG == 2:
        dma_stage2()

    def ln_block(i):
        rows = pl.ds(pl.multiple_of(i * R1, R1), R1)
        return _layernorm(x_s[rows, :].astype(F32), D)

    def tile(xn, col):
        return jnp.dot(xn, wqkv_s[:, col:col + LANES], preferred_element_type=F32)

    def proj_q(i, xn, dep=None):
        rows = pl.ds(pl.multiple_of(i * R1, R1), R1)
        lane = jax.lax.broadcasted_iota(I32, (R1, LANES), 1)
        zero = jnp.zeros((R1, LANES), BF16)
        prev = None
        for t in range(NTILE):
            q = tile(xn, t * LANES)
            if FOLD:
                q = q * C
            q = q.astype(BF16)
            if dep is not None and t == DEPT:
                q = jnp.where(never, dep, q)
            for h in range(H):
                th, lo, st = _head_geometry(h, DH)
                if st and th + 1 == t:
                    qsl = jnp.where(lane >= lo, prev, q)
                elif not st and th == t:
                    qsl = q
                else:
                    continue
                mask = ((lane - lo) & (LANES - 1)) < DH
                qm_s[h, rows, :] = jnp.where(mask, qsl, zero)
            prev = q

    def proj_k(i, xn):
        rows = pl.ds(pl.multiple_of(i * R1, R1), R1)
        lane = jax.lax.broadcasted_iota(I32, (R1, LANES), 1)
        prev = None
        for t in range(NTILE):
            k = tile(xn, D + t * LANES).astype(BF16)
            ks_s[t, rows, :] = k
            for n, h in enumerate(straddlers):
                th, lo, _ = _head_geometry(h, DH)
                if th + 1 == t:
                    ks_s[NTILE + n, rows, :] = jnp.where(lane >= lo, prev, k)
            prev = k

    def proj_v(i, xn):
        vt = _rb(jax.lax.dot_general(wvt_s[...], xn, NT, preferred_element_type=F32))
        sub = jax.lax.broadcasted_iota(I32, (VR, LANES), 0)
        for h in range(H):
            w0 = (h * DH) // 8 * 8
            o8 = h * DH - w0
            inhead = (sub >= o8) & (sub < o8 + DH)
            for c in range(R1 // LANES):
                win = vt[w0:w0 + VR, c * LANES:(c + 1) * LANES]
                vtw_s[h, i * (R1 // LANES) + c] = jnp.where(inhead, win, 1.0)

    def proj_block(i, xn, dep=None):
        proj_q(i, xn, dep)
        proj_k(i, xn)
        proj_v(i, xn)

    with scope("p1_ln0"):
        x_copy(0).wait()
        if STAG == 1:
            dma_stage2()
        xn0 = ln_block(0)
    with scope("p1_a"):
        x_copy(1).wait()
        wqkv_copy(0).wait()
        if STAG in (1, 2):
            dma_stage3()
        if STAG == 3:
            dma_stage2()
            dma_stage3()
        proj_q(0, xn0)
        xn1 = ln_block(1)
        proj_q(1, xn1)
    with scope("p1_b"):
        wqkv_copy(1).wait()
        wqkv_copy(2).wait()
        if STAG in (1, 2, 3):
            dma_stage4()
        wvt_s[...] = wqkv_s[:, 2 * D:3 * D].T
        proj_k(0, xn0)
        proj_k(1, xn1)
        proj_v(0, xn0)
        if NFIRST == 2:
            for i in range(2, N1):
                x_copy(i).wait()
            xn = ln_block(2)
        proj_v(1, xn1)
        if NFIRST == 3:
            x_copy(2).wait()
            xn = ln_block(2)

    if DEPT >= 0:
        w_late[0].wait()
        never = z_s[0] != 0

    zs = jnp.zeros((LANES, LANES), F32)
    for half in (s1a, s1b):
        for j in range(NQ):
            for r in range(0, S // 2 + 8, LANES):
                n = min(LANES, S // 2 + 8 - r)
                half[j, r:r + n, :] = zs[0:n]
    for j in range(NQ):
        m0[j] = zs[0:8]

    def proj_step(i, xn):
        for u in range(U1):
            b = 2 + i * U1 + u
            if NFIRST == 3:
                x_copy(b + 1).wait()
            xn_next = ln_block(b + 1)
            proj_block(b, xn, xn_next[:, 0:LANES] if DEPT >= 0 else None)
            xn = xn_next
        return xn

    with scope("p1_loop"):
        if U1 < N1 - 3:
            xn = jax.lax.fori_loop(0, (N1 - 3) // U1, proj_step, xn)
        else:
            xn = proj_step(0, xn)
    with scope("p1_last"):
        proj_block(N1 - 1, xn)

    NKT = S // LANES
    NQB = S // QB
    HK = NKT // 2
    s0 = (s0a, s0b)
    s1 = (s1a, s1b)
    if LATE:
        for c in w_late[1:]:
            c.start()
    if DEPT < 0:
        w_late[0].wait()
    off = pl.multiple_of(jnp.clip(z_s[0], 0, 1) * 8, 8)

    def head_slab(h):
        col = h * DH
        t = col >> 7
        lo = col & (LANES - 1)
        return jnp.where(lo + DH > LANES, NTILE + t, t)

    def qk_start(h, qb):
        return dict(slab=head_slab(h), h=h, q0=pl.multiple_of(qb * QB, QB), ms=[None] * NQ)

    def qk_chunk(st, s_ref, kc):
        q = qm_s[st["h"], pl.ds(st["q0"], QB), :]
        k = ks_s[st["slab"], kc * LANES:(kc + 1) * LANES, :]
        s = jax.lax.dot_general(k, q, NT, preferred_element_type=F32)
        for j in range(NQ):
            sj = s[:, j * LANES:(j + 1) * LANES]
            s_ref[kc // HK][j, (kc % HK) * LANES:(kc % HK + 1) * LANES, :] = sj
            pm = jnp.max(sj.reshape(LANES // 8, 8, LANES), axis=0)
            st["ms"][j] = pm if st["ms"][j] is None else jnp.maximum(st["ms"][j], pm)

    def qk_finish(st):
        return [jnp.broadcast_to(jnp.max(st["ms"][j], axis=0, keepdims=True), (8, LANES))
                for j in range(NQ)]

    def ep_chunk(st, s_ref, kc):
        vt = vtw_s[st["h"], kc]
        for j in range(NQ):
            s = s_ref[kc // HK][j, pl.ds(off + (kc % HK) * LANES, LANES), :]
            e = s.reshape(LANES // 8, 8, LANES) - st["m"][j][None]
            p = jnp.exp2(e if FOLD else e * C)
            p = p.reshape(LANES, LANES).astype(BF16)
            d = jnp.dot(vt, p, preferred_element_type=F32)
            st["acc"][j] = d if st["acc"][j] is None else st["acc"][j] + d

    def ep_finish(st):
        pair, parity, qb = st["pair"], st["parity"], st["qb"]
        for j in range(NQ):
            acc = st["acc"][j]
            q0 = pl.multiple_of(qb * QB + j * LANES, LANES)
            if parity == 0:
                l = acc[DH:DH + 1, :]
                ot_s[pair, 0:DH, pl.ds(q0, LANES)] = acc[0:DH, :] * (1.0 / l)
            else:
                l = acc[0:1, :]
                ot_s[pair, DH:2 * DH, pl.ds(q0, LANES)] = acc[VR - DH:VR, :] * (1.0 / l)

    NB = 8
    NITEMS = H * NQB
    sbuf = (s0, s1)

    def item_of(g2, parity):
        return g2 // NQB, parity, g2 % NQB

    def ep_state(item, m):
        pair, par, qb = item
        return dict(pair=pair, parity=par, qb=qb, h=2 * pair + par, m=m, acc=[None] * NQ)

    def att_step(i, carry):
        items = []
        for b in range(NB + 1):
            g2 = i * (NB // 2) + ((b - 1) >> 1)
            if b == 0:
                g2 = jnp.where(g2 < 0, NITEMS // 2 - 1, g2)
            items.append(item_of(g2, (b + 1) % 2))
        mx = {0: [m0[j] for j in range(NQ)]}
        qst = {}
        est = {}
        for t in range(NB * NKT + LAG):
            if t < NB * NKT:
                b, kc = divmod(t, NKT)
                if kc == 0:
                    pair, par, qb = items[b + 1]
                    qst = qk_start(2 * pair + par, qb)
                qk_chunk(qst, sbuf[b % 2], kc)
                if kc == NKT - 1:
                    mx[b + 1] = qk_finish(qst)
            u = t - LAG
            if u >= 0:
                b, kc = divmod(u, NKT)
                if kc == 0:
                    est = ep_state(items[b], mx[b])
                ep_chunk(est, sbuf[(b + 1) % 2], kc)
                if kc == NKT - 1:
                    ep_finish(est)
        for j in range(NQ):
            m0[j] = mx[NB][j]
        return carry

    with scope('att'):
        jax.lax.fori_loop(0, NITEMS // NB, att_step, 0)

    def last_item():
        est = ep_state(item_of(NITEMS // 2 - 1, 1), [m0[j] for j in range(NQ)])
        for kc in range(NKT):
            ep_chunk(est, sbuf[1], kc)
        ep_finish(est)

    bv_s[...] = jnp.full((8, LANES), -jnp.inf, F32)
    bi_s[...] = jnp.zeros((8, LANES), I32)
    w_late[1].wait()
    w_late[2].wait()
    wr = wr_s[...].astype(F32).reshape(1, D)

    def out_copy(i):
        rows = pl.ds(pl.multiple_of(i * R3, R3), R3)
        return pltpu.make_async_copy(out_s.at[rows], out_hbm.at[rows], sem_o.at[i])

    def epi_mm(i):
        rows = pl.ds(pl.multiple_of(i * R3, R3), R3)
        oT = ot_s[:, :, rows].reshape(D, R3).astype(BF16)
        return jnp.dot(oT.T, wo_s[...], preferred_element_type=F32)

    def epi_post(i, attn, state):
        r0 = pl.multiple_of(i * R3, R3)
        rows = pl.ds(r0, R3)
        h = _rb(x_s[rows, :].astype(F32) + _rb(attn))
        hn = _layernorm(h, D).astype(F32)
        r = jnp.sum(hn * wr, axis=-1, keepdims=True)
        h_s[rows, :] = h
        hn_s[rows, :] = hn
        out_s[rows, :] = (h + hn).astype(BF16)
        out_copy(i).start()
        bv, bi = state
        lane = jax.lax.broadcasted_iota(I32, (8, LANES), 1)
        sub = jax.lax.broadcasted_iota(I32, (8, LANES), 0)
        pos = ((lane >> 3) << 3) + sub
        for n, rv in enumerate(_compact(r)):
            rv = _rb(rv)
            upd = rv > bv
            bv = jnp.where(upd, rv, bv)
            bi = jnp.where(upd, pos + (r0 + n * LANES), bi)
        return bv, bi

    SK3 = int(os.environ.get("KSK3", "1"))

    LASTPOS = int(os.environ.get("KLASTPOS", "1"))

    def epi_step(i, carry):
        state = (bv_s[...], bi_s[...])
        mms = {}
        for u in range(U3 + SK3):
            if u == LASTPOS:
                last_item()
            if u < U3:
                mms[u] = epi_mm(i * U3 + u)
            if u - SK3 >= 0:
                state = epi_post(i * U3 + u - SK3, mms.pop(u - SK3), state)
        bv_s[...] = state[0]
        bi_s[...] = state[1]
        return carry

    with scope("p3"):
        if N3 // U3 > 1:
            jax.lax.fori_loop(0, N3 // U3, epi_step, 0)
        else:
            epi_step(0, 0)

    with scope('p4'):
        bv = bv_s[...]
        bi = bi_s[...]
        vmax = jnp.max(bv)
        idx = jnp.min(jnp.where(bv == vmax, bi, S))
        idx = jnp.clip(idx, 0, S - 1)
        xsel = hn_s[pl.ds(idx, 1), :]
        hsel = h_s[pl.ds(idx, 1), :]
        xb = jnp.broadcast_to(xsel, (16, D)).astype(BF16)
        w_late[3].wait()
        w_late[4].wait()
        g = _rb(jnp.dot(xb, wg_s[...], preferred_element_type=F32))
        u = _rb(jnp.dot(xb, wu_s[...], preferred_element_type=F32))
        act = _rb(g * jax.nn.sigmoid(g))
        t = (act * u).astype(BF16)
        w_late[5].wait()
        y = _rb(jnp.dot(t, wd_s[...], preferred_element_type=F32))
        rsel = _rb(jax.nn.sigmoid(jnp.full((16, LANES), vmax, F32)))
        y = _rb(y * rsel[:, 0:1])
        newrow = (hsel + _rb(xsel + y)).astype(BF16)
        base = pl.multiple_of((idx // 16) * 16, 16)
        rowid = jax.lax.broadcasted_iota(I32, (16, D), 0) + base
        old = out_s[pl.ds(base, 16), :]
        patch_s[...] = jnp.where(rowid == idx, newrow, old)
    with scope('p4_dma'):
        for i in range(N3):
            out_copy(i).wait()
        patch = pltpu.make_async_copy(patch_s, out_hbm.at[pl.ds(base, 16)], sem_o.at[N3])
        patch.start()
        patch.wait()


def build(S, D, FF):
    DH = D // H
    n_str = len([h for h in range(H) if _head_geometry(h, DH)[2]])
    scratch = [
        pltpu.SMEM((1,), I32),
        pltpu.VMEM((S, D), BF16),
        pltpu.VMEM((D, 3 * D), BF16),
        pltpu.VMEM((D, D), BF16),
        pltpu.VMEM((D,) if WR1D else (1, D), BF16),
        pltpu.VMEM((D, FF), BF16),
        pltpu.VMEM((D, FF), BF16),
        pltpu.VMEM((FF, D), BF16),
        pltpu.VMEM((S, D), BF16),
        pltpu.VMEM((16, D), BF16),
        pltpu.VMEM((D, D), BF16),
        pltpu.VMEM((H, S, LANES), BF16),
        pltpu.VMEM((D // LANES + n_str, S, LANES), BF16),
        pltpu.VMEM((H, S // LANES, VR, LANES), F32),
        pltpu.VMEM((NQ, S // 2 + 8, LANES), F32),
        pltpu.VMEM((NQ, S // 2 + 8, LANES), F32),
        pltpu.VMEM((NQ, S // 2 + 8, LANES), F32),
        pltpu.VMEM((NQ, S // 2 + 8, LANES), F32),
        pltpu.VMEM((NQ, 8, LANES), F32),
        pltpu.VMEM((NQ, 8, LANES), F32),
        pltpu.VMEM((H // 2, 2 * DH, S), F32),
        pltpu.VMEM((S, D), F32),
        pltpu.VMEM((S, D), F32),
        pltpu.VMEM((8, LANES), F32),
        pltpu.VMEM((8, LANES), I32),
        pltpu.SemaphoreType.DMA((S // R1,)),
        pltpu.SemaphoreType.DMA((9,)),
        pltpu.SemaphoreType.DMA((S // R3 + 1,)),
    ]
    anyspec = pl.BlockSpec(memory_space=pl.ANY)
    return pl.pallas_call(
        functools.partial(kernel, S=S, D=D, DH=DH, FF=FF),
        out_shape=jax.ShapeDtypeStruct((S, D), BF16),
        in_specs=[anyspec] * 8,
        out_specs=anyspec,
        scratch_shapes=scratch,
        compiler_params=pltpu.CompilerParams(vmem_limit_bytes=120 * 1024 * 1024),
        name="fused_block",
    )


@jax.jit
def pallas_sequential_preLN__mha_block__moe_arch_mod__prompt_kernel(
        A_x, A_wqkv, A_wo, B_x, B_w_r, B_w_gate, B_w_up, B_w_down):
    del B_x
    B, S, D = A_x.shape
    FF = B_w_gate.shape[1]
    out = build(S, D, FF)(
        jnp.zeros((1,), I32),
        A_x.reshape(S, D), A_wqkv, A_wo, B_w_r if WR1D else B_w_r.reshape(1, D), B_w_gate, B_w_up, B_w_down)
    return out.reshape(B, S, D)
```

```python
import functools

import jax
import jax.numpy as jnp
import numpy as np
from jax.experimental import pallas as pl
from jax.experimental.pallas import tpu as pltpu

F32 = jnp.float32
BF16 = jnp.bfloat16
I32 = jnp.int32
U32 = jnp.uint32

H = 32
LANES = 128
QB = 512
NQ = QB // LANES
VR = 24
NB = 8
LAG = 1
R1 = 256
U1 = 2
R3 = 128

NT = (((1,), (1,)), ((), ()))


def _rb(x):
    return x.astype(BF16).astype(F32)


def _compact(col):
    r = col.shape[0]
    v = jnp.broadcast_to(col, (r, LANES)).reshape(r // 8, 8, LANES)
    lane = jax.lax.broadcasted_iota(I32, (8, LANES), 1)
    out = []
    for n in range(r // LANES):
        parts = [v[16 * n + g] for g in range(16)]
        width = 8
        while len(parts) > 1:
            m = (lane & width) != 0
            parts = [jnp.where(m, parts[i + 1], parts[i]) for i in range(0, len(parts), 2)]
            width *= 2
        out.append(parts[0])
    return out


def _expand(vregs):
    rows = [jnp.broadcast_to(c[:, 8 * g:8 * g + 1], (8, LANES)) for c in vregs for g in range(16)]
    return jnp.concatenate(rows, axis=0)


def _layernorm(xf, d):
    inv_d = np.float32(1.0 / d)
    mean = jnp.sum(xf, axis=-1, keepdims=True) * inv_d
    c = xf - mean
    ssq = jnp.sum(c * c, axis=-1, keepdims=True)
    eps = np.float32(np.asarray(1e-5, dtype=jnp.bfloat16))
    rcp = _expand([1.0 / _rb(jnp.sqrt(_rb(_rb(v * inv_d) + eps))) for v in _compact(ssq)])
    dev = _rb(xf - _rb(mean))
    rcp = jnp.concatenate([rcp] * (d // LANES), axis=1)
    return (dev * rcp).astype(BF16)


def _head_geometry(h, dh):
    col = h * dh
    tile, lo = col // LANES, col % LANES
    return tile, lo, lo + dh > LANES


def _q_groups(h, dh):
    t, lo, _ = _head_geometry(h, dh)
    out = []
    for g in range(LANES // 16):
        r0 = 16 * g
        keep = [(((r0 + r) - lo) % LANES) < dh for r in range(16)]
        if any(keep):
            a = keep.index(True)
            b = a + sum(keep)
            assert all(keep[a:b])
            out.append((g, t * LANES + r0 if r0 + 15 >= lo else (t + 1) * LANES + r0, a, b))
    return out


def _kernel(z_hbm, x_hbm, wqkv_hbm, wo_hbm, wr_hbm, wg_hbm, wu_hbm, wd_hbm,
            out_hbm,
            z_s, x_s, wqkv_s, wo_s, wr_s, wg_s, wu_s, wd_s, out_s, patch_s,
            wqt_s, wvt_s, qm_s, ks_s, vtw_s, s0a, s0b, s1a, s1b, m_s, ot_s, h_s, hn_s,
            sem_x, sem_w, sem_o,
            *, S, D, DH):
    NTILE = D // LANES
    N1 = S // R1
    N3 = S // R3
    NKT = S // LANES
    NQB = S // QB
    HK = NKT // 2
    NITEMS = H * NQB
    straddlers = [h for h in range(H) if _head_geometry(h, DH)[2]]
    scale = float(np.float32(np.asarray(DH ** -0.5, dtype=jnp.bfloat16)))
    C = np.float32(scale * np.log2(np.e))

    def x_copy(i):
        rows = pl.ds(i * R1, R1)
        return pltpu.make_async_copy(x_hbm.at[rows], x_s.at[rows], sem_x.at[i])

    def wqkv_copy(p):
        cols = pl.ds(p * D, D)
        return pltpu.make_async_copy(wqkv_hbm.at[:, cols], wqkv_s.at[:, cols], sem_w.at[p])

    z_copy = pltpu.make_async_copy(z_hbm, z_s, sem_w.at[3])
    wo_copy = pltpu.make_async_copy(wo_hbm, wo_s, sem_w.at[4])
    wr_copy = pltpu.make_async_copy(wr_hbm, wr_s, sem_w.at[5])
    wg_copy = pltpu.make_async_copy(wg_hbm, wg_s, sem_w.at[6])
    wu_copy = pltpu.make_async_copy(wu_hbm, wu_s, sem_w.at[7])
    wd_copy = pltpu.make_async_copy(wd_hbm, wd_s, sem_w.at[8])

    x_copy(0).start()
    x_copy(1).start()
    wqkv_copy(1).start()

    def ln_block(i):
        rows = pl.ds(pl.multiple_of(i * R1, R1), R1)
        return _layernorm(x_s[rows, :].astype(F32), D)

    def zero_q(c, carry):
        zero = jnp.zeros((8, LANES), U32)
        for h in range(H):
            used = [g for g, _, _, _ in _q_groups(h, DH)]
            for g in range(LANES // 16):
                if g not in used:
                    qm_s[h, c, 8 * g:8 * g + 8, :] = zero
        return carry

    def proj_q(i, xn):
        qt = jax.lax.dot_general(wqt_s[...], xn, NT, preferred_element_type=F32)
        sub = jax.lax.broadcasted_iota(I32, (16, LANES), 0)
        zero = jnp.zeros((16, LANES), BF16)
        for c in range(R1 // LANES):
            blks = {}
            for h in range(H):
                for g, src, a, b in _q_groups(h, DH):
                    if src not in blks:
                        blks[src] = (qt[src:src + 16, c * LANES:(c + 1) * LANES] * C).astype(BF16)
                    blk = blks[src]
                    if (a, b) != (0, 16):
                        blk = jnp.where((sub >= a) & (sub < b), blk, zero)
                    qm_s[h, i * (R1 // LANES) + c, 8 * g:8 * g + 8, :] = pltpu.bitcast(blk, U32)

    def proj_k(i, xn):
        rows = pl.ds(pl.multiple_of(i * (R1 // 2), R1 // 2), R1 // 2)
        lane = jax.lax.broadcasted_iota(I32, (R1, LANES), 1)
        prev = None
        for t in range(NTILE):
            w = wqkv_s[:, D + t * LANES:D + (t + 1) * LANES]
            k = jnp.dot(xn, w, preferred_element_type=F32).astype(BF16)
            ks_s[t, rows, :] = pltpu.bitcast(k, U32)
            for n, h in enumerate(straddlers):
                th, lo, _ = _head_geometry(h, DH)
                if th + 1 == t:
                    ks_s[NTILE + n, rows, :] = pltpu.bitcast(jnp.where(lane >= lo, prev, k), U32)
            prev = k

    def proj_v(i, xn):
        vt = _rb(jax.lax.dot_general(wvt_s[...], xn, NT, preferred_element_type=F32))
        sub = jax.lax.broadcasted_iota(I32, (VR, LANES), 0)
        for h in range(H):
            w0 = (h * DH) // 8 * 8
            o8 = h * DH - w0
            inhead = (sub >= o8) & (sub < o8 + DH)
            for c in range(R1 // LANES):
                win = vt[w0:w0 + VR, c * LANES:(c + 1) * LANES]
                vtw_s[h, i * (R1 // LANES) + c] = jnp.where(inhead, win, 1.0)

    jax.lax.fori_loop(0, S // LANES, zero_q, 0)
    x_copy(0).wait()
    wqkv_copy(0).start()
    wqkv_copy(2).start()
    xn0 = ln_block(0)

    x_copy(1).wait()
    wqkv_copy(1).wait()
    for i in range(2, N1):
        x_copy(i).start()
    proj_k(0, xn0)
    xn1 = ln_block(1)
    proj_k(1, xn1)

    wqkv_copy(0).wait()
    wqkv_copy(2).wait()
    z_copy.start()
    wqt_s[...] = wqkv_s[:, 0:D].T
    wvt_s[...] = wqkv_s[:, 2 * D:3 * D].T
    proj_q(0, xn0)
    proj_q(1, xn1)
    proj_v(0, xn0)
    for i in range(2, N1):
        x_copy(i).wait()
    xn2 = ln_block(2)
    proj_v(1, xn1)

    zs = jnp.zeros((LANES, LANES), F32)
    for half in (s1a, s1b):
        for j in range(NQ):
            for r in range(0, S // 2 + 8, LANES):
                n = min(LANES, S // 2 + 8 - r)
                half[j, r:r + n, :] = zs[0:n]
    for j in range(NQ):
        m_s[j] = zs[0:8]

    def proj_step(i, xn):
        for u in range(U1):
            b = 2 + i * U1 + u
            xn_next = ln_block(jnp.minimum(b + 1, N1 - 1) if u == U1 - 1 else b + 1)
            proj_q(b, xn)
            proj_k(b, xn)
            proj_v(b, xn)
            xn = xn_next
        return xn

    jax.lax.fori_loop(0, (N1 - 2) // U1, proj_step, xn2)

    for c in (wo_copy, wr_copy, wg_copy, wu_copy, wd_copy):
        c.start()
    z_copy.wait()
    off = pl.multiple_of(jnp.clip(z_s[0], 0, 1) * 8, 8)
    sbuf = ((s0a, s0b), (s1a, s1b))

    def qk_start(item):
        pair, parity, qb = item
        h = 2 * pair + parity
        col = h * DH
        t = col >> 7
        slab = jnp.where((col & (LANES - 1)) + DH > LANES, NTILE + t, t)
        return dict(slab=slab, h=h, qt0=qb * NQ, ms=[None] * NQ)

    def qk_chunk(st, s_ref, kc):
        k = pltpu.bitcast(ks_s[st["slab"], kc * (LANES // 2):(kc + 1) * (LANES // 2), :], BF16)
        ss = [jnp.dot(k, pltpu.bitcast(qm_s[st["h"], st["qt0"] + j], BF16), preferred_element_type=F32)
              for j in range(NQ)]
        for j in range(NQ):
            s_ref[kc // HK][j, (kc % HK) * LANES:(kc % HK + 1) * LANES, :] = ss[j]
            pm = jnp.max(ss[j].reshape(LANES // 8, 8, LANES), axis=0)
            st["ms"][j] = pm if st["ms"][j] is None else jnp.maximum(st["ms"][j], pm)

    def qk_finish(st):
        return [jnp.broadcast_to(jnp.max(st["ms"][j], axis=0, keepdims=True), (8, LANES))
                for j in range(NQ)]

    def ep_start(item, m):
        pair, parity, qb = item
        return dict(pair=pair, parity=parity, qb=qb, h=2 * pair + parity, m=m, acc=[None] * NQ)

    def ep_chunk(st, s_ref, kc):
        vt = vtw_s[st["h"], kc]
        for j in range(NQ):
            s = s_ref[kc // HK][j, pl.ds(off + (kc % HK) * LANES, LANES), :]
            p = jnp.exp2(s.reshape(LANES // 8, 8, LANES) - st["m"][j][None])
            d = jnp.dot(vt, p.reshape(LANES, LANES).astype(BF16), preferred_element_type=F32)
            st["acc"][j] = d if st["acc"][j] is None else st["acc"][j] + d

    def ep_finish(st):
        for j in range(NQ):
            acc = st["acc"][j]
            cols = pl.ds(pl.multiple_of(st["qb"] * QB + j * LANES, LANES), LANES)
            if st["parity"] == 0:
                ot_s[st["pair"], 0:DH, cols] = acc[0:DH, :] * (1.0 / acc[DH:DH + 1, :])
            else:
                ot_s[st["pair"], DH:2 * DH, cols] = acc[VR - DH:VR, :] * (1.0 / acc[0:1, :])

    def item_of(g2, parity):
        return g2 // NQB, parity, g2 % NQB

    def att_step(i, carry):
        items = []
        for b in range(NB + 1):
            g2 = i * (NB // 2) + ((b - 1) >> 1)
            if b == 0:
                g2 = jnp.where(g2 < 0, NITEMS // 2 - 1, g2)
            items.append(item_of(g2, (b + 1) % 2))
        mx = {0: [m_s[j] for j in range(NQ)]}
        qst = est = None
        for t in range(NB * NKT + LAG):
            if t < NB * NKT:
                b, kc = divmod(t, NKT)
                if kc == 0:
                    qst = qk_start(items[b + 1])
                qk_chunk(qst, sbuf[b % 2], kc)
                if kc == NKT - 1:
                    mx[b + 1] = qk_finish(qst)
            if t >= LAG:
                b, kc = divmod(t - LAG, NKT)
                if kc == 0:
                    est = ep_start(items[b], mx[b])
                ep_chunk(est, sbuf[(b + 1) % 2], kc)
                if kc == NKT - 1:
                    ep_finish(est)
        for j in range(NQ):
            m_s[j] = mx[NB][j]
        return carry

    jax.lax.fori_loop(0, NITEMS // NB, att_step, 0)

    wo_copy.wait()
    wr_copy.wait()
    wr = wr_s[...].astype(F32).reshape(1, D)

    def out_copy(i):
        rows = pl.ds(i * R3, R3)
        return pltpu.make_async_copy(out_s.at[rows], out_hbm.at[rows], sem_o.at[i])

    def epi_mm(i):
        ot = ot_s[:, :, pl.ds(i * R3, R3)].reshape(D, R3).astype(BF16)
        return jnp.dot(ot.T, wo_s[...], preferred_element_type=F32)

    def epi_post(i, attn, best):
        rows = pl.ds(i * R3, R3)
        h = _rb(x_s[rows, :].astype(F32) + _rb(attn))
        hn = _layernorm(h, D).astype(F32)
        r = jnp.sum(hn * wr, axis=-1, keepdims=True)
        h_s[rows, :] = h
        hn_s[rows, :] = hn
        out_s[rows, :] = (h + hn).astype(BF16)
        out_copy(i).start()
        bv, bi = best
        lane = jax.lax.broadcasted_iota(I32, (8, LANES), 1)
        sub = jax.lax.broadcasted_iota(I32, (8, LANES), 0)
        pos = ((lane >> 3) << 3) + sub
        for n, rv in enumerate(_compact(r)):
            rv = _rb(rv)
            upd = rv > bv
            bv = jnp.where(upd, rv, bv)
            bi = jnp.where(upd, pos + (i * R3 + n * LANES), bi)
        return bv, bi

    wg_copy.wait()
    wu_copy.wait()
    wd_copy.wait()
    last = ep_start(item_of(NITEMS // 2 - 1, 1), [m_s[j] for j in range(NQ)])
    for kc in range(NKT):
        ep_chunk(last, sbuf[1], kc)
    ep_finish(last)

    best = (jnp.full((8, LANES), -jnp.inf, F32), jnp.zeros((8, LANES), I32))
    attn = epi_mm(0)
    for i in range(N3):
        nxt = epi_mm(i + 1) if i + 1 < N3 else None
        best = epi_post(i, attn, best)
        attn = nxt

    bv, bi = best
    vmax = jnp.max(bv)
    idx = jnp.clip(jnp.min(jnp.where(bv == vmax, bi, S)), 0, S - 1)
    xsel = hn_s[pl.ds(idx, 1), :]
    hsel = h_s[pl.ds(idx, 1), :]
    xb = jnp.broadcast_to(xsel, (8, D))
    g = _rb(jnp.dot(xb, wg_s[...], preferred_element_type=F32))
    u = _rb(jnp.dot(xb, wu_s[...], preferred_element_type=F32))
    act = _rb(g * jax.nn.sigmoid(g))
    y = _rb(jnp.dot(_rb(act * u), wd_s[...], preferred_element_type=F32))
    rsel = _rb(jax.nn.sigmoid(jnp.full((8, LANES), vmax, F32)))
    y = _rb(y * rsel[:, 0:1])
    newrow = hsel + _rb(xsel + y)
    newrow = jnp.concatenate([newrow, newrow], axis=0).astype(BF16)
    base = pl.multiple_of((idx // 16) * 16, 16)
    rowid = jax.lax.broadcasted_iota(I32, (16, D), 0) + base
    patch_s[...] = jnp.where(rowid == idx, newrow, out_s[pl.ds(base, 16), :])
    for i in range(N3):
        out_copy(i).wait()
    patch = pltpu.make_async_copy(patch_s, out_hbm.at[pl.ds(base, 16)], sem_o.at[N3])
    patch.start()
    patch.wait()


@jax.jit
def pallas_sequential_preLN__mha_block__moe_arch_mod__prompt_kernel(
    A_x: jax.Array,
    A_wqkv: jax.Array,
    A_wo: jax.Array,
    B_x: jax.Array,
    B_w_r: jax.Array,
    B_w_gate: jax.Array,
    B_w_up: jax.Array,
    B_w_down: jax.Array,
):
    del B_x
    B, S, D = A_x.shape
    FF = B_w_gate.shape[1]
    DH = D // H
    assert B == 1 and DH == 20 and S % (2 * QB) == 0 and (S // R1 - 2) % U1 == 0
    n_slabs = D // LANES + sum(_head_geometry(h, DH)[2] for h in range(H))
    scores = pltpu.VMEM((NQ, S // 2 + 8, LANES), F32)
    scratch = [
        pltpu.SMEM((1,), I32),
        pltpu.VMEM((S, D), BF16),
        pltpu.VMEM((D, 3 * D), BF16),
        pltpu.VMEM((D, D), BF16),
        pltpu.VMEM((D,), BF16),
        pltpu.VMEM((D, FF), BF16),
        pltpu.VMEM((D, FF), BF16),
        pltpu.VMEM((FF, D), BF16),
        pltpu.VMEM((S, D), BF16),
        pltpu.VMEM((16, D), BF16),
        pltpu.VMEM((D, D), BF16),
        pltpu.VMEM((D, D), BF16),
        pltpu.VMEM((H, S // LANES, LANES // 2, LANES), U32),
        pltpu.VMEM((n_slabs, S // 2, LANES), U32),
        pltpu.VMEM((H, S // LANES, VR, LANES), F32),
        scores, scores, scores, scores,
        pltpu.VMEM((NQ, 8, LANES), F32),
        pltpu.VMEM((H // 2, 2 * DH, S), F32),
        pltpu.VMEM((S, D), F32),
        pltpu.VMEM((S, D), F32),
        pltpu.SemaphoreType.DMA((S // R1,)),
        pltpu.SemaphoreType.DMA((9,)),
        pltpu.SemaphoreType.DMA((S // R3 + 1,)),
    ]
    anyspec = pl.BlockSpec(memory_space=pl.ANY)
    out = pl.pallas_call(
        functools.partial(_kernel, S=S, D=D, DH=DH),
        out_shape=jax.ShapeDtypeStruct((S, D), BF16),
        in_specs=[anyspec] * 8,
        out_specs=anyspec,
        scratch_shapes=scratch,
        compiler_params=pltpu.CompilerParams(vmem_limit_bytes=120 * 1024 * 1024),
        name="fused_block",
    )(jnp.zeros((1,), I32), A_x.reshape(S, D), A_wqkv, A_wo, B_w_r, B_w_gate, B_w_up, B_w_down)
    return out.reshape(B, S, D)
```
